```python
import os as _os
_os.environ.setdefault("JAX_PLATFORMS", "cpu")
import jax
import jax.numpy as jnp

def _softmax(x, axis=-1):
    return jax.nn.softmax(x, axis=axis)
def _gelu(x):
    return jax.nn.gelu(x, approximate=True)
def _silu(x):
    return jax.nn.silu(x)
def _sigmoid(x):
    return jax.nn.sigmoid(x)
def _layernorm(x, axis=-1, eps=1e-5):
    m = jnp.mean(x, axis=axis, keepdims=True)
    v = jnp.var(x, axis=axis, keepdims=True)
    return (x - m) / jnp.sqrt(v + eps)
def _scatter_add(tgt, idx, src, axis=0):
    return tgt.at[idx].add(src)
def _segment_sum(src, seg, n):
    return jax.ops.segment_sum(src, seg, n)
class _Rng:
    def __init__(self, key):
        self._k = key
    def _next(self):
        self._k, sub = jax.random.split(self._k)
        return sub
    def normal(self, shape):
        return jax.random.normal(self._next(), shape, dtype=jnp.bfloat16)
    def randint(self, lo, hi, shape):
        return jax.random.randint(self._next(), shape, lo, hi, dtype=jnp.int32)
    def uniform(self, shape, lo=0.0, hi=1.0):
        return jax.random.uniform(self._next(), shape, jnp.bfloat16, lo, hi)
    def permutation(self, n):
        return jax.random.permutation(self._next(), n)


kernel_name = 'gated_mix__compressed_kv_cla__ssm_conv_h3__prompt'

def setup_inputs():
    _rng = _Rng(jax.random.key(int.from_bytes(__import__("os").urandom(4), "little")))
    _w = (lambda a: (lambda t: t.astype(jnp.bfloat16) if jnp.issubdtype(t.dtype, jnp.floating) else t)(jnp.asarray(a)))
    def _A_setup():
        B, H, Sq, Sk, D, M = 1, 32, 2048, 2048, 128, 1024
        Dc = 4 * D
        return {
            "x": _w((lambda *s: _rng.normal(s) * 0.05)(B, Sq, M)),
            "c_kv": _w((lambda *s: _rng.normal(s) * 0.8)(B, Sk, Dc)),
            "w_q": _w((lambda *s: _rng.normal(s) * 3.2)(M, H, D) * (M ** -0.5)),
            "w_uk": _w((lambda *s: _rng.normal(s) * 3.2)(Dc, H, D) * (Dc ** -0.5)),
            "w_uv": _w((lambda *s: _rng.normal(s) * 0.8)(Dc, H, D) * (Dc ** -0.5)),
            "w_o": _w((lambda *s: _rng.normal(s) * 0.8)(H, D, M) * ((H * D) ** -0.5)),
        }
    _A_in = _A_setup()

    def _B_setup():
        B, S, D = 1, 2048, 1024
        ks = 4
        return {
            "q": _w((lambda *s: _rng.normal(s) * 0.05)(B, S, D)),
            "k": _w((lambda *s: _rng.normal(s) * 0.8)(B, S, D)),
            "v": _w((lambda *s: _rng.normal(s) * 0.8)(B, S, D)),
            "shift_k": _w((lambda *s: _rng.normal(s) * 0.8)(D, ks) * 0.5),
            "ssm_k": _w((lambda *s: _rng.normal(s) * 0.8)(D, S) * (1.0 / S ** 0.5)),
            "ssm_D": _w((lambda *s: _rng.normal(s) * 0.8)(D)),
        }
    _B_in = _B_setup()

    return {
        "A_x": _A_in["x"],
        "A_c_kv": _A_in["c_kv"],
        "A_w_q": _A_in["w_q"],
        "A_w_uk": _A_in["w_uk"],
        "A_w_uv": _A_in["w_uv"],
        "A_w_o": _A_in["w_o"],
        "B_q": _B_in["q"],
        "B_k": _B_in["k"],
        "B_v": _B_in["v"],
        "B_shift_k": _B_in["shift_k"],
        "B_ssm_k": _B_in["ssm_k"],
        "B_ssm_D": _B_in["ssm_D"],
        "gate_w": _w((lambda *s: _rng.normal(s) * 0.05)(1024) * 16.0),
    }

def reference(A_x, A_c_kv, A_w_q, A_w_uk, A_w_uv, A_w_o, B_q, B_k, B_v, B_shift_k, B_ssm_k, B_ssm_D, gate_w):
    def _A_ref(x, c_kv, w_q, w_uk, w_uv, w_o):
        B, Sq, M = x.shape[0], x.shape[1], x.shape[2]
        Sk = c_kv.shape[1]
        H, D = w_q.shape[1], w_q.shape[2]
        q = jnp.einsum("bqm,mhd->bhqd", x, w_q)
        k = jnp.einsum("bkc,chd->bhkd", c_kv, w_uk)
        v = jnp.einsum("bkc,chd->bhkd", c_kv, w_uv)
        scores = jnp.einsum("bhqd,bhkd->bhqk", q, k) * (D ** -0.5)
        off = Sk - Sq
        qi = jnp.arange(Sq)[:, None]
        kj = jnp.arange(Sk)[None, :]
        cmask = kj <= (qi + off)
        scores = jnp.where(cmask[None, None], scores, -1e9)
        p = _softmax(scores, axis=-1)
        ctx = jnp.einsum("bhqk,bhkd->bhqd", p, v)
        return jnp.einsum("bhqd,hdm->bqm", ctx, w_o)

    def _B_ref(q, k, v, shift_k, ssm_k, ssm_D):
        B, S, D = q.shape
        ks = shift_k.shape[-1]
        k_pad = jnp.pad(k, ((0, 0), (ks - 1, 0), (0, 0)))
        k_shift = jnp.zeros_like(k)
        for t in range(ks):
            k_shift = k_shift + k_pad[:, t:t + S, :] * shift_k[:, ks - 1 - t][None, None, :]
        kv = k_shift * v
        L = 2 * S
        kv_pad = jnp.pad(kv, ((0, 0), (0, S), (0, 0)))
        kf_pad = jnp.pad(ssm_k, ((0, 0), (0, S)))
        kv_f = (lambda x, axes=(-2,-1): jnp.fft.rfft2(x.astype(jnp.float32), axes=axes))(kv_pad[:, None, :, :], axes=(1, 2))
        kf_f = (lambda x, axes=(-2,-1): jnp.fft.rfft2(x.astype(jnp.float32), axes=axes))(kf_pad[:, None, :], axes=(1, 2))
        kf_f = (lambda x, *d: x.transpose(*d))(kf_f, 1, 2, 0)
        y_f = kv_f * kf_f[None, :, :, :]
        y = (lambda x, s, axes=(-2,-1): jnp.fft.irfft2(x, s=s, axes=axes).astype(jnp.bfloat16))(y_f, (1, L), axes=(1, 2))[:, 0, :S, :]
        y = y + kv * ssm_D[None, None, :]
        return q * y

    x = A_x
    g = _sigmoid((x * gate_w).sum(-1, keepdims=True))
    a = _A_ref(x, A_c_kv, A_w_q, A_w_uk, A_w_uv, A_w_o)
    b = _B_ref(x, B_k, B_v, B_shift_k, B_ssm_k, B_ssm_D)
    return g * a + (1 - g) * b
```

```python
import functools
import math
import numpy as np
import jax
import jax.numpy as jnp
import jax.experimental.pallas as pl
import jax.experimental.pallas.tpu as pltpu

S = 2048
M = 1024
DC = 512
H = 32
D = 128
NSTEP = H // 2
HG = 8
NG = H // HG
PG = HG // 2
WR = 128
NP = (M + 2 * DC) // WR
KO, VO, QO = 0, DC, 2 * DC
TQ = 256
NB = S // TQ
SUB = TQ // 128
CH = 128
NCH = S // CH
CG = 128
Q4 = CH // 4
RT = 8
GR = 144
TAIL = "Q7 V7 Q0 O7 V0 Q1 O0 V1 Q2 O1 V2 Q3 O2 V3 Q4 O3 V4 Q5 O4 V5 Q6 O5 V6 O6s"
SCHED = "q0 h0 h1 h2 h3 h4 h5 h6 h7 h8 h9 h10 h11 h12 h13 h14 h15 Q0:u0,u1 k0 V0:u2,u3 Q1@6:u10,y1 q1 k1 V1:y3,u5 O0 Q2:y2,u4 q2 k2 V2:u6,u7 O1 Q3:y0,y5! q3 k3 V3:u8,u9 O2 Q4:y4,u14 q4 k4 V4:u12,u11 O3 Q5@6:u13,y7 q5 k5 V5:y8,y9 O4 Q6@10:u15,y6 q6 k6e V6:y12,y13 O5 Q7@6:y10,y11 q7g k7 V7@6 O6 y14 y15 O7"
QCUT = (0, 9, 13, 16)
QLAG = 2
OR = 128
PB = 512
SEM_GROUPS = ('wk0', 'wv0', 'dft sh sd gw sk0 bk0 bv0', 'wq0', 'wk1 wo0', 'wv1 wq1 wo1 sk1 bk1 bv1',
              'wk2 wv2 wq2 wo2 sk2 bk2 bv2 bk3 bv3 bk4 bv4 bk5 bv5 bk6 bv6 bk7 bv7 wk3 wv3 wq3')
CS0 = len(SEM_GROUPS)
XS0 = CS0 + S // PB
EARLY = {2: ((15, 4),), 3: ((14, 4),), 4: ((15, 5), (13, 2),), 5: ((14, 6), (12, 2),), 6: ((15, 10), (12, 6), (11, 9),), 7: ((14, 8), (13, 8),), 10: ((11, 11),)}
NT = (((1,), (1,)), ((), ()))
F32 = jnp.float32
BF16 = jnp.bfloat16
U32 = jnp.uint32


def _dft_mats():
    n = np.arange(CH)[None, :]
    fwd = []
    for p in range(2):
        ke = np.arange(0, CH, 2)[p * 32:(p + 1) * 32]
        ko = np.arange(1, CH, 2)[p * 32:(p + 1) * 32]
        k = np.concatenate([ke, ko])[:, None]
        th = 2.0 * np.pi * (k + 0.5) * n / (2 * CH)
        fwd.append(np.concatenate([np.cos(th), np.sin(th)], axis=0))
    fwd = np.stack(fwd)
    inv = np.transpose(fwd, (0, 2, 1)) / CH
    return np.concatenate([fwd, inv], axis=0).astype(np.float32)


def _after(tok, val):
    return jnp.where(tok != tok, tok, val)


def _kernel(x_hbm, c_hbm, wq_hbm, wuk_hbm, wuv_hbm, wo_hbm, bk_hbm, bv_hbm, sk_hbm, sh_hbm, sd_hbm, gw_hbm, dft_hbm,
            o_hbm,
            x_ref, c_ref, raw, wo_ref, bk_ref, bv_ref, sk_ref, sh_ref, sd_ref, gw_ref, dft_ref,
            acc_ref, y_ref, w_s, qn, kn, vn, g_ref, o_s, u_s, h_s, z_s, kv_s, tmp, sd1_ref, gw1_ref,
            sems, osems):
    copies = {}

    def add(name, src, dst):
        k = [n for n, grp in enumerate(SEM_GROUPS) if name in grp.split()][0]
        copies[name] = pltpu.make_async_copy(src, dst, sems.at[k])

    def c_copy(i):
        r = pl.ds(pl.multiple_of(i * PB, PB), PB)
        return pltpu.make_async_copy(c_hbm.at[r], c_ref.at[r], sems.at[CS0 + i])

    def x_copy(i):
        r = pl.ds(pl.multiple_of(i * PB, PB), PB)
        return pltpu.make_async_copy(x_hbm.at[r], x_ref.at[r], sems.at[XS0 + i])

    def w_add(g):
        cols = pl.ds(g * HG, HG)
        add('wk%d' % g, wuk_hbm.at[:, :, cols, :], raw.at[pl.ds(g * NP + KO // WR, DC // WR)])
        add('wv%d' % g, wuv_hbm.at[:, :, cols, :], raw.at[pl.ds(g * NP + VO // WR, DC // WR)])
        add('wq%d' % g, wq_hbm.at[:, :, cols, :], raw.at[pl.ds(g * NP + QO // WR, M // WR)])

    def ssm_add(tag, g0, g1):
        rows = pl.ds(g0 * CG, (g1 - g0) * CG)
        add('sk' + tag, sk_hbm.at[rows], sk_ref.at[rows])
        for g in range(g0, g1):
            add('bk%d' % g, bk_hbm.at[:, pl.ds(g * CG, CG)], bk_ref.at[g])
            add('bv%d' % g, bv_hbm.at[:, pl.ds(g * CG, CG)], bv_ref.at[g])

    def wo_add(tag, s0, s1):
        rows = pl.ds(s0 * 2 * D, (s1 - s0) * 2 * D)
        add('wo' + tag, wo_hbm.at[rows], wo_ref.at[rows])

    for g in range(NG):
        w_add(g)
    add('dft', dft_hbm, dft_ref)
    add('sh', sh_hbm, sh_ref)
    add('sd', sd_hbm, sd1_ref)
    add('gw', gw_hbm, gw1_ref)
    ssm_add('0', 0, 1)
    wo_add('0', 0, 1)
    wo_add('1', 1, 4)
    ssm_add('1', 1, 2)
    wo_add('2', 4, NSTEP)
    ssm_add('2', 2, M // CG)

    def start(*names):
        for n in names:
            copies[n].start()

    def wait(*names):
        for n in names:
            copies[n].wait()

    def out_copy(k):
        r = pl.ds(k * OR, OR)
        return pltpu.make_async_copy(o_s.at[r], o_hbm.at[r], osems.at[0])

    qscale = (D ** -0.5) * math.log2(math.e)
    P = functools.partial

    TS = 2 * HG

    def relayout_stage(p, k, n):
        R = WR // n
        v = raw[p, k * R:(k + 1) * R].reshape(R * HG, D)
        w_s[TS, k * R * PG:(k + 1) * R * PG, :] = pltpu.bitcast(v, U32)

    def relayout_pair(p, jp):
        slot = pl.multiple_of(((p // NP) % 2) * HG, HG)
        r0 = pl.multiple_of((p % NP) * (WR // 2), WR // 2)
        a = w_s[TS, pl.ds(jp, WR // 2, stride=2 * PG), :]
        b = w_s[TS, pl.ds(PG + jp, WR // 2, stride=2 * PG), :]
        w_s[slot + 2 * jp, pl.ds(r0, WR // 2), :] = (a & U32(0xFFFF)) | (b << 16)
        w_s[slot + 2 * jp + 1, pl.ds(r0, WR // 2), :] = (a >> 16) | (b & U32(0xFFFF0000))

    def weight(h, off, n):
        return pltpu.bitcast(w_s[h, off // 2:(off + n) // 2, :], BF16)

    def qproj(rows, h0, between=(), tie=None):
        xr = x_ref[rows, :]
        for e in range(2):
            q = jnp.dot(xr, weight(h0 + e, QO, M), preferred_element_type=F32) * qscale
            if tie is not None and e == 1:
                q = jnp.concatenate([q[:-RT], _after(tie, q[-RT:])], axis=0)
            qn[e, rows, :] = q.astype(BF16)
            for f in between[e:e + 1]:
                f()

    def kvproj(rows, h0, between=()):
        cr = c_ref[rows, :]
        for e in range(2):
            kn[e, rows, :] = jnp.dot(cr, weight(h0 + e, KO, DC), preferred_element_type=F32).astype(BF16)
            for f in between[2 * e:2 * e + 1]:
                f()
            vn[e, rows, :] = jnp.dot(cr, weight(h0 + e, VO, DC), preferred_element_type=F32).astype(BF16)
            for f in between[2 * e + 1:2 * e + 2]:
                f()

    def gate(rows, n, tok0):
        gw = _after(jnp.concatenate([tok0[0:1]] * (M // 128), axis=1), gw_ref[...].astype(F32))
        z = jnp.sum(x_ref[rows, :].astype(F32) * gw, axis=-1, keepdims=True)
        g = jnp.broadcast_to(1.0 / (1.0 + jnp.exp(-z)), (n, 128))
        g_ref[rows, :] = g
        return functools.reduce(jnp.add, [g[k * RT:(k + 1) * RT] for k in range(n // RT)])

    def ssm_hraw(a, c0, half):
        return jax.lax.dot_general(dft_ref[half], sk_ref[pl.ds(c0, CG), a * CH:(a + 1) * CH], NT,
                                   preferred_element_type=F32)

    def ssm_hmix(hh, pr):
        if pr is None:
            return hh[:2 * Q4], hh[2 * Q4:]
        hr = jnp.concatenate([hh[0:Q4] + pr[2 * Q4:3 * Q4], hh[Q4:2 * Q4] - pr[3 * Q4:]], axis=0)
        hi = jnp.concatenate([hh[2 * Q4:3 * Q4] - pr[0:Q4], hh[3 * Q4:] + pr[Q4:2 * Q4]], axis=0)
        return hr, hi

    def ssm_kv(a, g, c0):
        cols = pl.ds(c0, CG)
        rows = slice(a * CH, (a + 1) * CH)
        k = bk_ref[g, rows, :].astype(F32)
        if a == 0:
            prev = jnp.zeros((8, CG), F32)
        else:
            prev = bk_ref[g, a * CH - 16:a * CH, :].astype(F32)[8:]
        ext = jnp.concatenate([prev, k], axis=0)
        sh = sh_ref[:, cols].astype(F32)
        kk = k * sh[0:1, :]
        for jj in range(1, 4):
            kk = kk + pltpu.roll(ext, jj, 0)[8:] * sh[jj:jj + 1, :]
        return kk * bv_ref[g, rows, :].astype(F32)

    def mac_chain(a, ks, ur, ui, hr, hi, tok, init=None):
        zr = zi = None
        for k in ks:
            tr = ur(k) * hr(a - k) - ui(k) * hi(a - k)
            ti = ur(k) * hi(a - k) + ui(k) * hr(a - k)
            if zr is None:
                if tok[0] is not None:
                    tr, ti = _after(tok[0], tr), _after(tok[1], ti)
                zr, zi = (tr, ti) if init is None else (init[0] + tr, init[1] + ti)
            else:
                zr, zi = zr + tr, zi + ti
        return zr, zi

    def step_body(step, last, eh=None):
        mult = pl.multiple_of
        heads = [eh] if last else [0, 1]
        NH = len(heads)
        nxt = step + 1
        hn0 = ((nxt // PG) % 2) * HG + 2 * (nxt % PG)
        half = nxt % 2
        c0 = None if last else mult((nxt // 2) * CG, CG)

        row = jax.lax.broadcasted_iota(jnp.int32, (128, 128), 0)
        col = jax.lax.broadcasted_iota(jnp.int32, (128, 128), 1)
        tri = col <= row

        ks = [[kn[h, j * 128:(j + 1) * 128, :] for j in range(NCH)] for h in heads]
        vs = [[vn[h, j * 128:(j + 1) * 128, :] for j in range(NCH)] for h in heads]
        qs = {}

        def qk_tile(e, i, j, s):
            t = max(0, j - i * SUB)
            if (e, i, t) not in qs:
                qs[e, i, t] = qn[heads[e], i * TQ + t * 128:(i + 1) * TQ, :]
            sj = jax.lax.dot_general(qs[e, i, t], ks[e][j], NT, preferred_element_type=F32)
            for u in range(t, SUB):
                piece = sj[(u - t) * 128:(u - t + 1) * 128]
                if j == i * SUB + u:
                    piece = jnp.where(tri, piece, -1e30)
                s[u][j] = piece

        def rowmax(s):
            ms = []
            for u in range(SUB):
                mx = functools.reduce(jnp.maximum, list(s[u].values()))
                ms.append(jnp.max(mx, axis=-1, keepdims=True))
            return ms

        def pv_tile(e, i, j, s, ms, accs, os_):
            t = max(0, j - i * SUB)
            ps = []
            for u in range(t, SUB):
                pt = jnp.exp2(s[u][j] - ms[u])
                if accs[u] is None:
                    accs[u] = pt
                else:
                    accs[u] = accs[u] + pt
                    pt = jnp.minimum(pt, accs[u])
                ps.append(pt)
            pj = jnp.concatenate(ps, axis=0).astype(BF16)
            oj = jnp.dot(pj, vs[e][j], preferred_element_type=F32)
            for u in range(t, SUB):
                piece = oj[(u - t) * 128:(u - t + 1) * 128]
                os_[u] = piece if os_[u] is None else os_[u] + piece

        def normalize(accs, os_):
            outs = []
            for u in range(SUB):
                l = jnp.sum(_after(os_[u], accs[u]), axis=-1, keepdims=True)
                r0 = pl.reciprocal(l, approx=True)
                r1 = r0 * (2.0 - l * r0)
                outs.append(os_[u] * r1)
            return jnp.concatenate(outs, axis=0)

        outs = {}

        def oproj(i, split=False):
            r = slice(i * TQ, (i + 1) * TQ)
            if not last:
                wo = wo_ref[pl.ds(mult(step * 2 * D, 2 * D), 2 * D), :]
                o = jnp.concatenate(outs[i], axis=1).astype(BF16)
                acc_ref[r, :] += jnp.dot(o, wo, preferred_element_type=F32)
            else:
                wo = wo_ref[pl.ds(mult((step * 2 + eh) * D, D), D), :]
                n = TQ // OR if split else 1
                R = TQ // n
                for k in range(n):
                    r = slice(i * TQ + k * R, i * TQ + (k + 1) * R)
                    o = outs[i][0][k * R:(k + 1) * R].astype(BF16)
                    a = acc_ref[r, :] + jnp.dot(o, wo, preferred_element_type=F32)
                    acc_ref[r, :] = a
                    g = jnp.concatenate([g_ref[r, :]] * (M // 128), axis=1)
                    b = x_ref[r, :].astype(F32) * jnp.concatenate([y_ref[n_, r, :] for n_ in range(M // CG)], axis=1)
                    o_s[r, :] = (b + g * (a - b)).astype(BF16)

                    @pl.when(eh == 1)
                    def _():
                        for kk in range(R // OR):
                            out_copy((i * TQ + k * R) // OR + kk).start()

        hraw = [None] * NCH
        hr = [None] * NCH
        hi = [None] * NCH
        us = [None] * NCH
        kvf = [None] * NCH

        def ssm_h(a):
            hraw[a] = ssm_hraw(a, c0, half)
            hr[a], hi[a] = ssm_hmix(hraw[a], hraw[a - 1] if a else None)

        def ssm_u(a):
            kvf[a] = ssm_kv(a, nxt // 2, c0)
            us[a] = jnp.dot(dft_ref[half], kvf[a].astype(BF16), preferred_element_type=F32)

        part = {}

        def ssm_mac(a, k1, tok):
            k0, init = part.get(a, (0, [None] * (2 * Q4 // RT)))
            res = []
            for r in range(2 * Q4 // RT):
                rr = slice(r * RT, (r + 1) * RT)
                ri = slice(2 * Q4 + r * RT, 2 * Q4 + (r + 1) * RT)
                tok = mac_chain(a, range(k0, k1), lambda k: us[k][rr], lambda k: us[k][ri],
                                lambda k: hr[k][rr], lambda k: hi[k][rr], tok, init[r])
                res.append(tok)
            part[a] = (k1, res)
            return tok

        def ssm_out(a, tok0=None):
            tok = [tok0, tok0]
            for a2, k1 in EARLY.get(a, ()):
                tok = ssm_mac(a2, k1, tok)
            ssm_mac(a, a + 1, tok)
            zrs = [z[0] for z in part[a][1]]
            zis = [z[1] for z in part[a][1]]
            z = jnp.concatenate(zrs + zis, axis=0).astype(BF16)
            y = jnp.dot(dft_ref[2 + half], z, preferred_element_type=F32)
            y = y + kvf[a].astype(BF16).astype(F32) * (0.5 * sd_ref[:, pl.ds(c0, CG)].astype(F32))
            rows = slice(a * CH, (a + 1) * CH)
            old = jnp.where(half == 1, y_ref[nxt // 2, rows, :], 0.0)
            y_ref[nxt // 2, rows, :] = old + y

        def phase(i, tile_fn, side, nb=2):
            full = [(e, j) for e in range(NH) for j in range(i * SUB + 1)]
            for e, j in full[:nb]:
                tile_fn(e, j)
            for e in range(NH):
                tile_fn(e, i * SUB + 1)
            for f in side:
                f()
            for e, j in full[nb:]:
                tile_fn(e, j)

        sc = {}

        def qk_phase(i, side, nb=2):
            sc[i] = [[{} for _ in range(SUB)] for _ in range(NH)]
            phase(i, lambda e, j: qk_tile(e, i, j, sc[i][e]), side, nb)

        def pv_phase(i, side, nb=2):
            ms = [rowmax(sc[i][e]) for e in range(NH)]
            accs = [[None] * SUB for _ in range(NH)]
            os_ = [[None] * SUB for _ in range(NH)]
            phase(i, lambda e, j: pv_tile(e, i, j, sc[i][e], ms[e], accs[e], os_[e]), side, nb)
            outs[i] = [normalize(accs[e], os_[e]) for e in range(NH)]

        if last:
            for item in TAIL.split():
                i = int(item[1])
                if item[0] == 'Q':
                    qk_phase(i, [])
                elif item[0] == 'V':
                    pv_phase(i, [])
                else:
                    oproj(i, item.endswith('s'))
            return

        pbase = jnp.where(step == 0, NP, jnp.minimum(NP + 4 * nxt, NG * NP - 4))
        rl = []
        for k in range(4):
            rl += [P(relayout_stage, pbase + k, kk, 4) for kk in range(4)]
            rl += [P(relayout_pair, pbase + k, jp) for jp in range(PG)]
        last_qk = [None]

        def ssm_op(tok):
            kind, a = tok[0], int(tok[1:].rstrip('!'))
            if kind == 'y':
                return P(ssm_out, a, sc[last_qk[0]][0][0][0][:RT] if tok.endswith('!') else None)
            return P({'h': ssm_h, 'u': ssm_u}[kind], a)

        for item in SCHED.split():
            op, _, side = item.partition(':')
            kind = op[0]
            if kind in 'huy':
                ssm_op(op)()
                continue
            i = int(op[1])
            rows = slice(i * TQ, (i + 1) * TQ)
            sides = [ssm_op(t) for t in side.split(',')] if side else []
            nb = int(op.partition('@')[2] or 2)
            if kind == 'Q':
                qk_phase(i, sides, nb)
                last_qk[0] = i
            elif kind == 'V':
                pv_phase(i, sides, nb)
            elif kind == 'O':
                oproj(i)
            elif kind == 'q':
                for e in range(2):
                    for t in range(SUB):
                        if (e, i, t) not in qs:
                            qs[e, i, t] = qn[e, i * TQ + t * 128:(i + 1) * TQ, :]
                tie = None
                if op.endswith('g'):
                    r0 = pl.multiple_of(jnp.minimum(step * GR, S - GR), 16)
                    tie = gate(pl.ds(r0, GR), GR, sc[last_qk[0]][0][0][0][:RT])
                qproj(rows, hn0, [rl.pop(0), rl.pop(0)], tie)
            elif kind == 'k':
                nop = lambda: None
                pat = {'': 'xx..', 'a': '.xx.', 'b': 'x.x.', 'c': '..xx', 'd': 'x..x', 'e': '.x.x'}[op[2:]]
                kvproj(rows, hn0, [rl.pop(0) if ch == 'x' else nop for ch in pat])

    start('wk0', 'wv0')
    for i in range(S // PB):
        c_copy(i).start()
    start('dft', 'sh', 'sd', 'gw', 'sk0', 'bk0', 'bv0', 'wq0')
    for i in range(S // PB):
        x_copy(i).start()
    for grp in SEM_GROUPS[4:]:
        start(*grp.split())

    def relayout_range(p0, p1):
        def body(t, carry):
            for k in range(2):
                p = p0 + 2 * t + k
                tmp[k, 0:WR * PG, :] = pltpu.bitcast(raw[p].reshape(WR * HG, D), U32)
            for k in range(2):
                p = p0 + 2 * t + k
                slot = pl.multiple_of(((p // NP) % 2) * HG, HG)
                r0 = pl.multiple_of((p % NP) * (WR // 2), WR // 2)
                for jp in range(PG):
                    a = tmp[k, pl.ds(jp, WR // 2, stride=2 * PG), :]
                    b = tmp[k, pl.ds(PG + jp, WR // 2, stride=2 * PG), :]
                    w_s[slot + 2 * jp, pl.ds(r0, WR // 2), :] = (a & U32(0xFFFF)) | (b << 16)
                    w_s[slot + 2 * jp + 1, pl.ds(r0, WR // 2), :] = (a >> 16) | (b & U32(0xFFFF0000))
            return carry
        jax.lax.fori_loop(0, (p1 - p0) // 2, body, 0)

    def prologue():
        def zero(i, carry):
            acc_ref[pl.ds(pl.multiple_of(i * 128, 128), 128), :] = jnp.zeros((128, M), F32)
            return carry
        jax.lax.fori_loop(0, S // 128, zero, 0)
        wait('wk0')
        relayout_range(0, 4)
        wait('wv0')
        relayout_range(4, 8)

        def kv_loop(i, carry):
            c_copy(i).wait()
            kvproj(pl.ds(pl.multiple_of(i * PB, PB), PB), 0)
            return carry
        jax.lax.fori_loop(0, S // PB, kv_loop, 0)

        wait('dft', 'sh', 'sd', 'gw', 'sk0', 'bk0', 'bv0')
        sd_ref[...] = sd1_ref[...].astype(F32).reshape(1, M).astype(BF16)
        gw_ref[...] = gw1_ref[...].astype(F32).reshape(1, M).astype(BF16)
        prev = None
        for a in range(NCH):
            hh = ssm_hraw(a, 0, 0)
            hr, hi = ssm_hmix(hh, prev)
            prev = hh
            h_s[a] = jnp.concatenate([hr, hi], axis=0)
            kv = ssm_kv(a, 0, 0).astype(BF16)
            kv_s[a] = kv.astype(F32)
            u_s[a] = jnp.dot(dft_ref[0], kv, preferred_element_type=F32)
        wait('wq0')
        relayout_range(8, 16)

        def q_loop(i, carry):
            x_copy(i).wait()

            def mac_tile(r, a0, a1, tok0):
                rr = pl.ds(pl.multiple_of(r * RT, RT), RT)
                ri = pl.ds(pl.multiple_of(2 * Q4 + r * RT, RT), RT)
                tok = [tok0, tok0]
                for a in range(a0, a1):
                    tok = mac_chain(a, range(a + 1), lambda k: u_s[k, rr, :], lambda k: u_s[k, ri, :],
                                    lambda k: h_s[k, rr, :], lambda k: h_s[k, ri, :], tok)
                    z_s[a, rr, :] = tok[0]
                    z_s[a, ri, :] = tok[1]
                return _after(tok[0], tok[1])

            QR = PB // 4
            rows = [pl.ds(pl.multiple_of(i * PB + k * QR, QR), QR) for k in range(4)]
            side = [P(mac_tile, 2 * i + t, a0, a1) for t in range(2) for a0, a1 in zip(QCUT[:-1], QCUT[1:])]
            pending = [None] * QLAG
            for k in range(4):
                xr = x_ref[rows[k], :]
                for e in range(2):
                    q = jnp.dot(xr, weight(e, QO, M), preferred_element_type=F32) * qscale
                    done = pending.pop(0)
                    if done is not None:
                        q = jnp.concatenate([q[:QR - RT], _after(done, q[QR - RT:])], axis=0)
                    qn[e, rows[k], :] = q.astype(BF16)
                    f = side.pop(0) if side else None
                    pending.append(f(q[:RT]) if f else None)
            return carry
        jax.lax.fori_loop(0, S // PB, q_loop, 0)
        for a in range(NCH):
            y = jnp.dot(dft_ref[2], z_s[a].astype(BF16), preferred_element_type=F32)
            y_ref[0, a * CH:(a + 1) * CH, :] = y + kv_s[a] * (0.5 * sd_ref[:, 0:CG].astype(F32))
        wait('wk1', 'wo0')

    def loop(step, carry):
        pl.when(step == 0)(prologue)

        @pl.when(step == 1)
        def _():
            wait('wv1', 'wq1', 'wo1', 'sk1', 'bk1', 'bv1')
            relayout_range(20, 24)

        @pl.when(step == 3)
        def _():
            wait(*SEM_GROUPS[6].split())
        step_body(step, False)
        return carry
    jax.lax.fori_loop(0, NSTEP - 1, loop, 0)

    def tail(eh, carry):
        step_body(NSTEP - 1, True, eh)
        return carry
    jax.lax.fori_loop(0, 2, tail, 0)
    for k in range(S // OR):
        out_copy(k).wait()


@jax.jit
def pallas_gated_mix__compressed_kv_cla__ssm_conv_h3__prompt_kernel(
    A_x, A_c_kv, A_w_q, A_w_uk, A_w_uv, A_w_o, B_q, B_k, B_v, B_shift_k, B_ssm_k, B_ssm_D, gate_w,
):
    del B_q
    dft = jnp.asarray(_dft_mats(), dtype=BF16)
    x = A_x.reshape(S, M)
    c = A_c_kv.reshape(S, DC)
    wq = A_w_q.reshape(M // WR, WR, H, D)
    wuk = A_w_uk.reshape(DC // WR, WR, H, D)
    wuv = A_w_uv.reshape(DC // WR, WR, H, D)
    wo = A_w_o.reshape(H * D, M)
    bk = B_k.reshape(S, M)
    bv = B_v.reshape(S, M)
    sh = B_shift_k.T
    spec = pltpu.VMEM((NCH, CH, CG), F32)
    out = pl.pallas_call(
        _kernel,
        in_specs=[pl.BlockSpec(memory_space=pl.ANY)] * 13,
        out_specs=pl.BlockSpec(memory_space=pl.ANY),
        out_shape=jax.ShapeDtypeStruct((S, M), BF16),
        scratch_shapes=[
            pltpu.VMEM((S, M), BF16),
            pltpu.VMEM((S, DC), BF16),
            pltpu.VMEM((NG * NP, WR, HG, D), BF16),
            pltpu.VMEM((H * D, M), BF16),
            pltpu.VMEM((M // CG, S, CG), BF16),
            pltpu.VMEM((M // CG, S, CG), BF16),
            pltpu.VMEM((M, S), BF16),
            pltpu.VMEM((4, M), BF16),
            pltpu.VMEM((1, M), BF16),
            pltpu.VMEM((1, M), BF16),
            pltpu.VMEM((4, CH, CH), BF16),
            pltpu.VMEM((S, M), F32),
            pltpu.VMEM((M // CG, S, CG), F32),
            pltpu.VMEM((2 * HG + 1, NP * WR // 2, D), U32),
            pltpu.VMEM((2, S, D), BF16),
            pltpu.VMEM((2, S, D), BF16),
            pltpu.VMEM((2, S, D), BF16),
            pltpu.VMEM((S, 128), F32),
            pltpu.VMEM((S, M), BF16),
            spec, spec, spec, spec,
            pltpu.VMEM((2, WR * PG + 32, D), U32),
            pltpu.VMEM((M,), BF16),
            pltpu.VMEM((M,), BF16),
            pltpu.SemaphoreType.DMA((XS0 + S // PB,)),
            pltpu.SemaphoreType.DMA((1,)),
        ],
        compiler_params=pltpu.CompilerParams(
            vmem_limit_bytes=120 * 1024 * 1024,
        ),
        name="gmix",
    )(x, c, wq, wuk, wuv, wo, bk, bv, B_ssm_k, sh, B_ssm_D, gate_w, dft)
    return out.reshape(1, S, M)
```
